```python
import os as _os
_os.environ.setdefault("JAX_PLATFORMS", "cpu")
import jax
import jax.numpy as jnp

def _softmax(x, axis=-1):
    return jax.nn.softmax(x, axis=axis)
def _gelu(x):
    return jax.nn.gelu(x, approximate=True)
def _silu(x):
    return jax.nn.silu(x)
def _sigmoid(x):
    return jax.nn.sigmoid(x)
def _layernorm(x, axis=-1, eps=1e-5):
    m = jnp.mean(x, axis=axis, keepdims=True)
    v = jnp.var(x, axis=axis, keepdims=True)
    return (x - m) / jnp.sqrt(v + eps)
def _scatter_add(tgt, idx, src, axis=0):
    return tgt.at[idx].add(src)
def _segment_sum(src, seg, n):
    return jax.ops.segment_sum(src, seg, n)
class _Rng:
    def __init__(self, key):
        self._k = key
    def _next(self):
        self._k, sub = jax.random.split(self._k)
        return sub
    def normal(self, shape):
        return jax.random.normal(self._next(), shape, dtype=jnp.bfloat16)
    def randint(self, lo, hi, shape):
        return jax.random.randint(self._next(), shape, lo, hi, dtype=jnp.int32)
    def uniform(self, shape, lo=0.0, hi=1.0):
        return jax.random.uniform(self._next(), shape, jnp.bfloat16, lo, hi)
    def permutation(self, n):
        return jax.random.permutation(self._next(), n)


kernel_name = 'gated_mix__mha_block_cached__swiglu_ffn__decode'

def setup_inputs():
    _rng = _Rng(jax.random.key(int.from_bytes(__import__("os").urandom(4), "little")))
    _w = (lambda a: (lambda t: t.astype(jnp.bfloat16) if jnp.issubdtype(t.dtype, jnp.floating) else t)(jnp.asarray(a)))
    def _A_setup():
        B, Sq, D = 4, 1, 512
        H, Sk, Dh = 32, 4096, 128
        return {
            "x": _w((lambda *s: _rng.normal(s) * 0.05)(B, Sq, D)),
            "k_cache": _w((lambda *s: _rng.normal(s) * 3.2)(B, H, Sk, Dh)),
            "v_cache": _w((lambda *s: _rng.normal(s) * 0.4)(B, H, Sk, Dh)),
            "wq": _w((lambda *s: _rng.normal(s) * 3.2)(D, H * Dh) * (D ** -0.5)),
            "wo": _w((lambda *s: _rng.normal(s) * 0.4)(H * Dh, D) * ((H * Dh) ** -0.5)),
        }
    _A_in = _A_setup()

    def _B_setup():
        B, S, D, F = 4, 1, 512, 1376
        return {
            "x": _w((lambda *s: _rng.normal(s) * 0.05)(B, S, D)),
            "w_gate": _w((lambda *s: _rng.normal(s) * 0.05)(D, F)),
            "w_up": _w((lambda *s: _rng.normal(s) * 0.05)(D, F)),
            "w_down": _w((lambda *s: _rng.normal(s) * 0.05)(F, D)),
        }
    _B_in = _B_setup()

    return {
        "A_x": _A_in["x"],
        "A_k_cache": _A_in["k_cache"],
        "A_v_cache": _A_in["v_cache"],
        "A_wq": _A_in["wq"],
        "A_wo": _A_in["wo"],
        "B_x": _B_in["x"],
        "B_w_gate": _B_in["w_gate"],
        "B_w_up": _B_in["w_up"],
        "B_w_down": _B_in["w_down"],
        "gate_w": _w((lambda *s: _rng.normal(s) * 0.05)(512) * 16.0),
    }

def reference(A_x, A_k_cache, A_v_cache, A_wq, A_wo, B_x, B_w_gate, B_w_up, B_w_down, gate_w):
    def _A_ref(x, k_cache, v_cache, wq, wo):
        B, Sq, D = x.shape
        H, Dh = 32, 128
        q = (lambda x, *d: x.transpose(*d))((x @ wq).reshape(B, Sq, H, Dh), 0, 2, 1, 3)
        scores = jnp.einsum("bhqd,bhkd->bhqk", q, k_cache) * (Dh ** -0.5)
        p = _softmax(scores, axis=-1)
        o = jnp.einsum("bhqk,bhkd->bhqd", p, v_cache)
        return (lambda x, *d: x.transpose(*d))(o, 0, 2, 1, 3).reshape(B, Sq, H * Dh) @ wo

    def _B_ref(x, w_gate, w_up, w_down):
        g = _silu(x @ w_gate)
        u = x @ w_up
        return (g * u) @ w_down

    x = A_x
    g = _sigmoid((x * gate_w).sum(-1, keepdims=True))
    a = _A_ref(x, A_k_cache, A_v_cache, A_wq, A_wo)
    b = _B_ref(x, B_w_gate, B_w_up, B_w_down)
    return g * a + (1 - g) * b
```

```python
import contextlib
import functools
import math

import jax
import jax.numpy as jnp
from jax import lax
from jax.experimental import pallas as pl
from jax.experimental.pallas import tpu as pltpu

B, D, H, SK, DH, F = 4, 512, 32, 4096, 128, 1376
T = 128
G = 8
NKB = SK // T
NBLK = (B * H // G) * NKB
NW = 8
FB = -(-F // DH)
FU = F // 32
EXP2_SCALE = (DH ** -0.5) * math.log2(math.e)
F32, BF16 = jnp.float32, jnp.bfloat16
NT = (((1,), (1,)), ((), ()))


def make(L=3, name="gm", nbc=True, prof=0,
         sched="c012@037 s3 d65 s4 d65 s5 d65 s6 d65 s7 d45",
         d0=72, d1=45, d3=45, dinit=0, low=''):
    RK, RV = L + 1, L + 2
    scope = lambda nm, lvl=1: jax.named_scope(name + "_" + nm) if prof >= lvl else contextlib.nullcontext()

    def kernel(x_hbm, k_hbm, v_hbm, wq_hbm, wo_hbm, wg_hbm, wu_hbm, wd_hbm, gw_hbm, o_ref,
               kbuf, vbuf, wq, wo, wg, wu, wd, xs, gs, q_all, o_all, ffn_acc,
               sem_a, sem_b, sem_s):
        row = lax.broadcasted_iota(jnp.int32, (G, DH), 0)
        mult = lambda v, m: v if isinstance(v, int) else pl.multiple_of(v, m)

        def kv_copies(n, slot, kslot, vslot, i):
            r0 = mult((n // NKB if isinstance(n, int) else n >> 5) * (G * SK) + (n & (NKB - 1)) * T + i * SK, T)
            return (pltpu.make_async_copy(k_hbm.at[pl.ds(r0, T)], kbuf.at[kslot, i], sem_a.at[slot, i]),
                    pltpu.make_async_copy(v_hbm.at[pl.ds(r0, T)], vbuf.at[vslot, i], sem_b.at[slot, i]))

        def wq_copies(j, slot, i):
            rows = pl.ds(mult(i * 64 + j * 8, 8), 8)
            rows_b = pl.ds(mult(((i + 4) % 8) * 64 + j * 8, 8), 8)
            ia, ib = (rows, pl.ds(0, 2048)), (rows_b, pl.ds(2048, 2048))
            return (pltpu.make_async_copy(wq_hbm.at[ia], wq.at[ia], sem_a.at[slot, i]),
                    pltpu.make_async_copy(wq_hbm.at[ib], wq.at[ib], sem_b.at[slot, i]))

        def wo_copies(j, slot, i):
            ra = pl.ds(mult((i % 4) * 1024 + j * DH + (i // 4) * 32, 32), 32)
            rb = pl.ds(mult(((i + 2) % 4) * 1024 + j * DH + 64 + (i // 4) * 32, 32), 32)
            return (pltpu.make_async_copy(wo_hbm.at[ra], wo.at[ra], sem_a.at[slot, i]),
                    pltpu.make_async_copy(wo_hbm.at[rb], wo.at[rb], sem_b.at[slot, i]))

        def ffn_copy(u, j, sem):
            src, dst = ((wg_hbm, wg), (wu_hbm, wu), (wd_hbm, wd))[u % 3]
            if u < 15:
                r = (u // 3) * 8 + j
            else:
                return None
            rows = pl.ds(mult(r * 32, 32), 32)
            return pltpu.make_async_copy(src.at[rows], dst.at[rows], sem)

        def ffn_copies(j, slot, i):
            return ffn_copy(2 * i, j, sem_a.at[slot, i]), ffn_copy(2 * i + 1, j, sem_b.at[slot, i])

        def start(copies, i=None):
            for prio, c in enumerate(copies):
                if c is not None:
                    c.start(priority=1 if str(i) in low else prio)

        def wait(copies):
            for c in copies[::-1]:
                if c is not None:
                    c.wait()

        tail_rows = pl.ds(40 * 32, F - 40 * 32)
        small = [pltpu.make_async_copy(x_hbm, xs, sem_s.at[0]),
                 pltpu.make_async_copy(gw_hbm, gs, sem_s.at[1]),
                 pltpu.make_async_copy(wg_hbm.at[tail_rows], wg.at[tail_rows], sem_s.at[2]),
                 pltpu.make_async_copy(wu_hbm.at[tail_rows], wu.at[tail_rows], sem_s.at[3]),
                 pltpu.make_async_copy(wd_hbm.at[tail_rows], wd.at[tail_rows], sem_s.at[4])]

        def wrap(s, k, R):
            if isinstance(s, int):
                return (s + k) % R
            s = s + k
            return jnp.where(s >= R, s - R, s)

        def first(t, c):
            for i in range(G):
                start(wq_copies(t, t, i))
                if dinit:
                    pl.delay(dinit)
            return c

        lax.fori_loop(0, L, first, 0)
        for c in small:
            c.start(priority=1)
        pad = pl.ds(F, FB * DH - F)
        for w in (wg, wu, wd):
            w[pad, :] = jnp.zeros((FB * DH - F, D), BF16)
        vbuf[RV - 1] = jnp.zeros((G, T, DH), BF16)
        ffn_acc[...] = jnp.zeros((G, D), F32)
        o_zero = ffn_acc[:B, :]

        def load_x8():
            x4 = xs[...].astype(F32)
            return jnp.concatenate([x4, x4], axis=0).astype(BF16)

        def phase1(t, slot):
            nslot = wrap(slot, L, RK)

            @pl.when(t < NW)
            def _():
                for i in range(G):
                    wait(wq_copies(t, slot, i))

            @pl.when(t == NW)
            def _():
                for c in small:
                    c.wait()

            @pl.when(t >= NW)
            def _():
                for i in range(G):
                    wait(ffn_copies(t - NW, slot, i))
                c = mult((t - NW) * (4 * DH), 4 * DH)
                q4 = jnp.dot(load_x8(), wq[:, pl.ds(c, 4 * DH)], preferred_element_type=F32)
                for hh in range(4):
                    q_all[pl.ds((t - NW) * 4 + hh, B, stride=H), :] = q4[:B, hh * DH:(hh + 1) * DH]

            def issue(fn):
                for i in range(G):
                    start(fn(i))

                    @pl.when(t < NW)
                    def _():
                        pl.delay(d0)

                    @pl.when(t >= NW)
                    def _():
                        pl.delay(d1)

            u = t + L
            pl.when(u < NW)(lambda: issue(lambda i: wq_copies(u, nslot, i)))
            pl.when((u >= NW) & (u < 2 * NW))(lambda: issue(lambda i: ffn_copies(u - NW, nslot, i)))
            pl.when(u >= 2 * NW)(lambda: issue(lambda i: kv_copies(u - 2 * NW, nslot, nslot, u - 2 * NW, i)))
            return wrap(slot, 1, RK)

        with scope("p1"):
            slot = lax.fori_loop(0, 2 * NW, phase1, jnp.int32(0))

        def softmax_step(m, lsum, s):
            m_new = jnp.maximum(m, jnp.max(s, axis=1, keepdims=True))
            alpha = jnp.exp2((m - m_new) * EXP2_SCALE)
            e = jnp.exp2((s - m_new) * EXP2_SCALE)
            return m_new, lsum * alpha + e, e.astype(BF16), alpha

        def pv_tile(p, sv, i, pv):
            oi = jnp.dot(p, vbuf[sv, i], preferred_element_type=F32)
            return oi if i == 0 else jnp.where(row == i, oi, pv)

        def finish_group(g, acc, lsum):
            o_all[pl.ds(mult(g * G, G), G), :] = acc / jnp.sum(lsum, axis=1, keepdims=True)

        def ffn_band(j):
            rows = pl.ds(mult(j * DH, DH), DH)
            x8 = load_x8()
            gate = lax.dot_general(x8, wg[rows, :], NT, preferred_element_type=F32)
            up = lax.dot_general(x8, wu[rows, :], NT, preferred_element_type=F32)
            hid = (gate * jax.nn.sigmoid(gate) * up).astype(BF16)
            ffn_acc[...] += jnp.dot(hid, wd[rows, :], preferred_element_type=F32)

        neg = jnp.full((G, DH), -jnp.inf, F32)
        zero = jnp.zeros((G, DH), F32)

        def attn(n, st, issue):
            sk, sv, m, lsum, acc, s_prev = st
            sv_cur = wrap(sv, 1, RV)
            skn, svn = wrap(sk, L, RK), wrap(sv, L + 1, RV)
            s = s_prev
            for op in (sched if "w" in sched else "w " + sched).split():
                if op[0] == "s":
                    with scope(op, 2):
                        start(issue(n + L, skn, svn, int(op[1])), int(op[1]))
                elif op[0] == "d":
                    pl.delay(int(op[1:]))
                elif op[0] == "w":
                    for i in range(G):
                        wait(kv_copies(n, sk, sk, sv_cur, i))
                else:
                    idx, pos = ([int(c) for c in part] for part in op[1:].split("@"))
                    do_k, do_v = op[0] in "ck", op[0] in "cv"
                    if do_v:
                        m, lsum, p, alpha = softmax_step(m, lsum, s_prev)
                    if do_k:
                        q = q_all[pl.ds(mult((n >> 5) * G, G), G), :].astype(BF16)
                    pv = None
                    for i in range(G + 1):
                        for j, ps in zip(idx, pos):
                            if ps == i:
                                start(issue(n + L, skn, svn, j), j)
                        if i < G:
                            if do_k:
                                si = lax.dot_general(q, kbuf[sk, i], NT, preferred_element_type=F32)
                                s = si if i == 0 else jnp.where(row == i, si, s)
                            if do_v:
                                pv = pv_tile(p, sv, i, pv)
                    if do_v:
                        acc = acc * alpha + pv
            first_blk = (n & (NKB - 1)) == 0

            @pl.when(first_blk & (n > 0))
            def _():
                finish_group((n >> 5) - 1, acc, lsum)

            m = jnp.where(first_blk, neg, m)
            lsum = jnp.where(first_blk, zero, lsum)
            acc = jnp.where(first_blk, zero, acc)
            return wrap(sk, 1, RK), sv_cur, m, lsum, acc, s

        def main(n, st):
            st = attn(n, st, lambda u, skn, svn, i: kv_copies(u, skn, skn, svn, i))
            pl.when(n < FB)(lambda: ffn_band(n))
            return st

        z0 = ffn_acc[:, :DH]
        st = (slot, jnp.int32(RV - 1), z0, z0, z0, z0)
        with scope("main"):
            st = lax.fori_loop(0, NBLK - L, main, st)
        with scope("p2b"):
            st = lax.fori_loop(NBLK - L, NBLK,
                               lambda n, st: attn(n, st, lambda u, skn, svn, i: wo_copies(u - NBLK, skn, i)), st)
        slot, sv, m, lsum, acc, s_prev = st
        m, lsum, p, alpha = softmax_step(m, lsum, s_prev)
        pv = None
        for i in range(G):
            pv = pv_tile(p, sv, i, pv)
        finish_group(B * H // G - 1, acc * alpha + pv, lsum)

        def phase3(j, st):
            slot, out = st
            for i in range(G):
                wait(wo_copies(j, slot, i))
            for hh in range(4):
                h = hh * 8 + j
                o = o_all[pl.ds(h, B, stride=H), :].astype(BF16)
                out = out + jnp.dot(o, wo[pl.ds(mult(h * DH, DH), DH), :], preferred_element_type=F32)

            @pl.when(j + L < NW)
            def _():
                for i in range(G):
                    start(wo_copies(j + L, wrap(slot, L, RK), i))
                    pl.delay(d3)
            return wrap(slot, 1, RK), out

        gw = gs[...].astype(F32)
        x4 = xs[...].astype(F32)
        prod = sum(x4[:, r * DH:(r + 1) * DH] * gw[r:r + 1, :] for r in range(D // DH))
        gate = jax.nn.sigmoid(jnp.sum(prod, axis=1, keepdims=True))
        with scope("p3"):
            _, a_out = lax.fori_loop(0, NW, phase3, (slot, o_zero))
        o_ref[...] = (gate * a_out + (1.0 - gate) * ffn_acc[:B, :]).astype(o_ref.dtype)

    hbm = pl.BlockSpec(memory_space=pltpu.HBM)
    call = pl.pallas_call(
        kernel, name=name,
        out_shape=jax.ShapeDtypeStruct((B, D), BF16),
        in_specs=[hbm] * 9,
        out_specs=pl.BlockSpec(memory_space=pltpu.VMEM),
        scratch_shapes=[
            pltpu.VMEM((RK, G, T, DH), BF16), pltpu.VMEM((RV, G, T, DH), BF16),
            pltpu.VMEM((D, H * DH), BF16), pltpu.VMEM((H * DH, D), BF16),
            pltpu.VMEM((FB * DH, D), BF16), pltpu.VMEM((FB * DH, D), BF16), pltpu.VMEM((FB * DH, D), BF16),
            pltpu.VMEM((B, D), BF16), pltpu.VMEM((D // DH, DH), BF16),
            pltpu.VMEM((B * H, DH), F32), pltpu.VMEM((B * H, DH), F32), pltpu.VMEM((G, D), F32),
            pltpu.SemaphoreType.DMA((RK, G)), pltpu.SemaphoreType.DMA((RK, G)),
            pltpu.SemaphoreType.DMA((5,)),
        ],
        compiler_params=pltpu.CompilerParams(vmem_limit_bytes=64 * 1024 * 1024, disable_bounds_checks=nbc),
    )

    def fn(A_x, A_k_cache, A_v_cache, A_wq, A_wo, B_x, B_w_gate, B_w_up, B_w_down, gate_w):
        out = call(A_x.reshape(B, D), A_k_cache.reshape(B * H * SK, DH), A_v_cache.reshape(B * H * SK, DH),
                   A_wq, A_wo, B_w_gate.T, B_w_up.T, B_w_down, gate_w.reshape(D // DH, DH))
        return out.reshape(B, 1, D)

    return jax.jit(fn)


_fn = make(**dict(sched='c012@058 s3 d50 s4 d50 s5 d50 s6 d50 s7 d30', d0=55, d1=30, d3=30))


@jax.jit
def pallas_gated_mix__mha_block_cached__swiglu_ffn__decode_kernel(A_x, A_k_cache, A_v_cache, A_wq, A_wo, B_x, B_w_gate, B_w_up, B_w_down, gate_w):
    return _fn(A_x, A_k_cache, A_v_cache, A_wq, A_wo, B_x, B_w_gate, B_w_up, B_w_down, gate_w)
```

```python
import contextlib
import functools
import math

import jax
import jax.numpy as jnp
from jax import lax
from jax.experimental import pallas as pl
from jax.experimental.pallas import tpu as pltpu

B, D, H, SK, DH, F = 4, 512, 32, 4096, 128, 1376
T = 128
G = 8
NKB = SK // T
NBLK = (B * H // G) * NKB
NW = 8
FB = -(-F // DH)
EXP2_SCALE = (DH ** -0.5) * math.log2(math.e)
F32, BF16 = jnp.float32, jnp.bfloat16
NT = (((1,), (1,)), ((), ()))


def make(L=3, name="gm", nbc=False, prof=0, sched="c0@0 s1 d46 s2 d46 s3 d46 s4 d46 s5 d46 s6 d46 s7 d30",
         d0=46, d1=46, d3=46, dinit=46, bc=True, perm="02461357", vpos=0, lastsplit=False, nsc=False, dm='delay'):
    RK, RV = L + 1, L + 2
    scope = lambda nm, lvl=1: jax.named_scope(name + "_" + nm) if prof >= lvl else contextlib.nullcontext()

    def kernel(x_hbm, k_hbm, v_hbm, wq_hbm, wo_hbm, wg_hbm, wu_hbm, wd_hbm, gw_hbm, o_ref,
               kbuf, vbuf, wq, wo, wg, wu, wd, xs, gs, q_all, o_all, ffn_acc,
               sem_a, sem_b, sem_s, tick, sem_t, sem_r):
        row = lax.broadcasted_iota(jnp.int32, (G, DH), 0)
        mult = lambda v, m: v if isinstance(v, int) else pl.multiple_of(v, m)
        copy = pltpu.make_async_copy

        def pause(ns):
            if dm == "delay":
                pl.delay(ns)
            elif dm[:3] == "dma":
                c = copy(tick.at[0], tick.at[1], sem_t)
                c.start(priority=int(dm[3]))
                c.wait()
            elif dm[:3] == "sem":
                for _ in range(int(dm[3:])):
                    pl.semaphore_signal(sem_r, 1)
                    pl.semaphore_wait(sem_r, 1)
            elif dm[:4] == "loop":
                def body(_, c):
                    tick[0] += 1.0
                    return c
                lax.fori_loop(0, int(dm[4:]), body, 0)

        def kv_block(n, slot, vslot):
            h0 = mult((n // NKB if isinstance(n, int) else n >> 5) * G, G)
            keys = pl.ds(mult((n & (NKB - 1)) * T, T), T)
            small = [copy(k_hbm.at[h0 + i, keys], kbuf.at[slot, i], sem_a.at[slot]) for i in map(int, perm)]
            return small, [copy(v_hbm.at[pl.ds(h0, G), keys], vbuf.at[vslot], sem_b.at[slot])]

        def wq_block(j, slot):
            rows = pl.ds(mult(j * 8, 8), 8)
            lo, hi = pl.ds(0, 2048), pl.ds(2048, 2048)
            small = [copy(wq_hbm.at[i, rows, lo], wq.at[i, rows, lo], sem_a.at[slot]) for i in range(G)]
            return small, [copy(wq_hbm.at[:, rows, hi], wq.at[:, rows, hi], sem_b.at[slot])]

        def wo_block(j, slot):
            part = lambda u, n: pl.ds(mult(j * DH + u * 32, 32), n)
            small = [copy(wo_hbm.at[i % 4, part(i // 4, 32)], wo.at[i % 4, part(i // 4, 32)], sem_a.at[slot])
                     for i in range(G)]
            return small, [copy(wo_hbm.at[:, part(u, 32)], wo.at[:, part(u, 32)], sem_b.at[slot]) for u in (2, 3)]

        def ffn_block(j, slot):
            rows = lambda u, n: pl.ds(mult(j * 160 + u * 32, 32), n)
            part = lambda src, dst, u, n, sem: copy(src.at[rows(u, n)], dst.at[rows(u, n)], sem.at[slot])
            small = [part(wg_hbm, wg, i // 2, 32, sem_a) if i % 2 == 0 or i > 5 else part(wd_hbm, wd, i // 2, 32, sem_a)
                     for i in (0, 1, 2, 3, 4, 5, 6, 8)]
            return small, [part(wu_hbm, wu, 0, 160, sem_b), part(wd_hbm, wd, 3, 64, sem_b)]

        def start(block, i):
            small, bulk = block
            small[i].start(priority=0)
            if i == vpos:
                for c in bulk:
                    c.start(priority=1)

        def wait(block):
            for c in block[1] + block[0]:
                c.wait()

        def wait_kv(slot, vslot):
            copy(vbuf.at[vslot], vbuf.at[vslot], sem_b.at[slot]).wait()
            copy(kbuf.at[slot], kbuf.at[slot], sem_a.at[slot]).wait()

        tail_rows = pl.ds(40 * 32, F - 40 * 32)
        extra = [copy(x_hbm, xs, sem_s.at[0]),
                 copy(gw_hbm, gs, sem_s.at[1]),
                 copy(wg_hbm.at[tail_rows], wg.at[tail_rows], sem_s.at[2]),
                 copy(wu_hbm.at[tail_rows], wu.at[tail_rows], sem_s.at[3]),
                 copy(wd_hbm.at[tail_rows], wd.at[tail_rows], sem_s.at[4])]

        def wrap(s, k, R):
            if isinstance(s, int):
                return (s + k) % R
            s = s + k
            return jnp.where(s >= R, s - R, s)

        tick[0] = jnp.zeros((8, 128), F32)
        for t in range(L):
            for c in wq_block(t, t)[1]:
                c.start(priority=1)
        for c in extra:
            c.start(priority=1)

        def first(t, c):
            for cp in wq_block(t, t)[0]:
                cp.start(priority=0)
                if dinit:
                    pause(dinit)
            return c

        lax.fori_loop(0, L, first, 0)
        pad = pl.ds(F, FB * DH - F)
        for w in (wg, wu, wd):
            w[pad, :] = jnp.zeros((FB * DH - F, D), BF16)
        vbuf[RV - 1] = jnp.zeros((G, T, DH), BF16)
        ffn_acc[...] = jnp.zeros((G, D), F32)
        o_zero = ffn_acc[:B, :]

        def load_x8():
            x4 = xs[...].astype(F32)
            return jnp.concatenate([x4, x4], axis=0).astype(BF16)

        def phase1(t, slot):
            nslot = wrap(slot, L, RK)

            @pl.when(t < NW)
            def _():
                wait(wq_block(t, slot))

            @pl.when(t == NW)
            def _():
                for c in extra:
                    c.wait()

            @pl.when(t >= NW)
            def _():
                wait(ffn_block(t - NW, slot))
                c = mult((t - NW) * (4 * DH), 4 * DH)
                w = wq[:, :, pl.ds(c, 4 * DH)].reshape(D, 4 * DH)
                q4 = jnp.dot(load_x8(), w, preferred_element_type=F32)
                for hh in range(4):
                    q_all[pl.ds((t - NW) * 4 + hh, B, stride=H), :] = q4[:B, hh * DH:(hh + 1) * DH]

            def issue(block):
                for i in range(G):
                    start(block, i)
                    if d0 == d1:
                        pause(d0)
                    else:
                        pl.when(t < NW)(lambda: pause(d0))
                        if i < G - 1:
                            pl.when(t >= NW)(lambda: pause(d1))

            u = t + L
            pl.when(u < NW)(lambda: issue(wq_block(u, nslot)))
            pl.when((u >= NW) & (u < 2 * NW))(lambda: issue(ffn_block(u - NW, nslot)))
            pl.when(u >= 2 * NW)(lambda: issue(kv_block(u - 2 * NW, nslot, nslot)))
            return wrap(slot, 1, RK)

        assert (2 * NW) % RK == 0 or True
        with scope("p1"):
            slot = lax.fori_loop(0, 2 * NW, phase1, jnp.int32(0))
        s0 = (2 * NW) % RK

        def softmax_step(m, lsum, s):
            m_new = jnp.maximum(m, jnp.max(s, axis=1, keepdims=True))
            alpha = jnp.exp2((m - m_new) * EXP2_SCALE)
            e = jnp.exp2((s - m_new) * EXP2_SCALE)
            return m_new, lsum * alpha + e, e.astype(BF16), alpha

        def tile(buf, slot, i):
            if bc:
                return pltpu.bitcast(buf.bitcast(jnp.uint32)[slot, i], BF16)
            return buf[slot, i]

        def pv_tile(p, sv, i, pv):
            oi = jnp.dot(p, tile(vbuf, sv, i), preferred_element_type=F32)
            return oi if i == 0 else jnp.where(row == i, oi, pv)

        def finish_group(g, acc, lsum):
            o_all[pl.ds(mult(g * G, G), G), :] = acc / jnp.sum(lsum, axis=1, keepdims=True)

        def ffn_band(j):
            rows = pl.ds(mult(j * DH, DH), DH)
            x8 = load_x8()
            gate = lax.dot_general(x8, wg[rows, :], NT, preferred_element_type=F32)
            up = lax.dot_general(x8, wu[rows, :], NT, preferred_element_type=F32)
            hid = (gate * jax.nn.sigmoid(gate) * up).astype(BF16)
            ffn_acc[...] += jnp.dot(hid, wd[rows, :], preferred_element_type=F32)

        neg = jnp.full((G, DH), -jnp.inf, F32)
        zero = jnp.zeros((G, DH), F32)

        def attn(n, st, issue):
            sk, sv, m, lsum, acc, s_prev = st
            sv_cur = wrap(sv, 1, RV)
            nxt = issue(n + L, wrap(sk, L, RK), wrap(sv, L + 1, RV))
            wait_kv(sk, sv_cur)
            s = s_prev
            for op in sched.split():
                if op[0] == "s":
                    with scope(op, 2):
                        start(nxt, int(op[1]))
                elif op[0] == "d":
                    pause(int(op[1:]))
                else:
                    idx, pos = ([int(c) for c in part] for part in op[1:].split("@"))
                    do_k, do_v = op[0] in "ck", op[0] in "cv"
                    if do_v:
                        m, lsum, p, alpha = softmax_step(m, lsum, s_prev)
                    if do_k:
                        q = q_all[pl.ds(mult((n >> 5) * G, G), G), :].astype(BF16)
                    pv = None
                    for i in range(G + 1):
                        for j, ps in zip(idx, pos):
                            if ps == i:
                                start(nxt, j)
                        if i < G:
                            if do_k:
                                si = lax.dot_general(q, tile(kbuf, sk, i), NT, preferred_element_type=F32)
                                s = si if i == 0 else jnp.where(row == i, si, s)
                            if do_v:
                                pv = pv_tile(p, sv, i, pv)
                    if do_v:
                        acc = acc * alpha + pv
            first_blk = (n & (NKB - 1)) == 0

            @pl.when(first_blk & (n > 0))
            def _():
                finish_group((n >> 5) - 1, acc, lsum)

            m = jnp.where(first_blk, neg, m)
            lsum = jnp.where(first_blk, zero, lsum)
            acc = jnp.where(first_blk, zero, acc)
            return wrap(sk, 1, RK), sv_cur, m, lsum, acc, s

        def main(n, st):
            st = attn(n, st, kv_block)
            pl.when(((n & (NKB - 1)) == NKB // 2) & (n < FB * NKB))(lambda: ffn_band(n >> 5))
            return st

        z0 = ffn_acc[:, :DH]
        assert s0 == 0
        st = (slot, jnp.int32(RV - 1), z0, z0, z0, z0)
        with scope("main"):
            st = lax.fori_loop(0, NBLK - L, main, st)
        with scope("p2b"):
            st = lax.fori_loop(NBLK - L, NBLK,
                               lambda n, st: attn(n, st, lambda u, skn, svn: wo_block(u - NBLK, skn)), st)
        slot, sv, m, lsum, acc, s_prev = st
        m, lsum, p, alpha = softmax_step(m, lsum, s_prev)
        pv = None
        for i in range(G):
            pv = pv_tile(p, sv, i, pv)
        finish_group(B * H // G - 1, acc * alpha + pv, lsum)

        def phase3(j, st):
            slot, out = st
            wait(wo_block(j, slot))
            for hh in range(4):
                o = o_all[pl.ds(hh * 8 + j, B, stride=H), :].astype(BF16)
                out = out + jnp.dot(o, wo[hh, pl.ds(mult(j * DH, DH), DH), :], preferred_element_type=F32)

            @pl.when(j + L < NW)
            def _():
                nxt = wo_block(j + L, wrap(slot, L, RK))
                for i in range(G):
                    start(nxt, i)
                    if i < G - 1:
                        pause(d3)
            return wrap(slot, 1, RK), out

        gw = gs[...].astype(F32)
        x4 = xs[...].astype(F32)
        prod = sum(x4[:, r * DH:(r + 1) * DH] * gw[r:r + 1, :] for r in range(D // DH))
        gate = jax.nn.sigmoid(jnp.sum(prod, axis=1, keepdims=True))
        with scope("p3"):
            _, a_out = lax.fori_loop(0, NW, phase3, (slot, o_zero))
        o_ref[...] = (gate * a_out + (1.0 - gate) * ffn_acc[:B, :]).astype(o_ref.dtype)

    hbm = pl.BlockSpec(memory_space=pltpu.HBM)
    call = pl.pallas_call(
        kernel, name=name,
        out_shape=jax.ShapeDtypeStruct((B, D), BF16),
        in_specs=[hbm] * 9,
        out_specs=pl.BlockSpec(memory_space=pltpu.VMEM),
        scratch_shapes=[
            pltpu.VMEM((RK, G, T, DH), BF16), pltpu.VMEM((RV, G, T, DH), BF16),
            pltpu.VMEM((8, D // 8, H * DH), BF16), pltpu.VMEM((4, H * DH // 4, D), BF16),
            pltpu.VMEM((FB * DH, D), BF16), pltpu.VMEM((FB * DH, D), BF16), pltpu.VMEM((FB * DH, D), BF16),
            pltpu.VMEM((B, D), BF16), pltpu.VMEM((D // DH, DH), BF16),
            pltpu.VMEM((B * H, DH), F32), pltpu.VMEM((B * H, DH), F32), pltpu.VMEM((G, D), F32),
            pltpu.SemaphoreType.DMA((RK,)), pltpu.SemaphoreType.DMA((RK,)),
            pltpu.SemaphoreType.DMA((5,)),
            pltpu.VMEM((2, 8, 128), F32), pltpu.SemaphoreType.DMA, pltpu.SemaphoreType.REGULAR,
        ],
        compiler_params=pltpu.CompilerParams(vmem_limit_bytes=64 * 1024 * 1024, disable_bounds_checks=nbc, disable_semaphore_checks=nsc),
    )

    def fn(A_x, A_k_cache, A_v_cache, A_wq, A_wo, B_x, B_w_gate, B_w_up, B_w_down, gate_w):
        out = call(A_x.reshape(B, D), A_k_cache.reshape(B * H, SK, DH), A_v_cache.reshape(B * H, SK, DH),
                   A_wq.reshape(8, D // 8, H * DH), A_wo.reshape(4, H * DH // 4, D),
                   B_w_gate.T, B_w_up.T, B_w_down, gate_w.reshape(D // DH, DH))
        return out.reshape(B, 1, D)

    return jax.jit(fn)


_fn = make(**dict(nsc=True, bc=False))


@jax.jit
def pallas_gated_mix__mha_block_cached__swiglu_ffn__decode_kernel(A_x, A_k_cache, A_v_cache, A_wq, A_wo, B_x, B_w_gate, B_w_up, B_w_down, gate_w):
    return _fn(A_x, A_k_cache, A_v_cache, A_wq, A_wo, B_x, B_w_gate, B_w_up, B_w_down, gate_w)
```

```python
import math

import jax
import jax.numpy as jnp
from jax import lax
from jax.experimental import pallas as pl
from jax.experimental.pallas import tpu as pltpu

B, D, H, SK, DH, F = 4, 512, 32, 4096, 128, 1376

T = 128
G = 8
KEY_BLOCKS = SK // T
GROUPS = B * H // G
KV_BLOCKS = GROUPS * KEY_BLOCKS
W_BLOCKS = 8
FFN_ROWS = 160
FFN_BANDS = -(-F // DH)

DEPTH = 3
SLOTS = 4
V_SLOTS = 8
PAUSE_NS = 50
FIRST_PAUSE_NS = 70

EXP2_SCALE = DH ** -0.5 * math.log2(math.e)
F32, BF16 = jnp.float32, jnp.bfloat16


def _hint(v, m):
    return v if isinstance(v, int) else pl.multiple_of(v, m)


def _dot(a, b):
    return jnp.dot(a, b, preferred_element_type=F32)


def _dot_nt(a, b):
    return lax.dot_general(a, b, (((1,), (1,)), ((), ())), preferred_element_type=F32)


def _kernel(x_hbm, k_hbm, v_hbm, wq_hbm, wo_hbm, wg_hbm, wu_hbm, wd_hbm, gw_hbm, o_ref,
            k_buf, v_buf, wq, wo, wg, wu, wd, x_ref, gw_ref, q_all, o_all, ffn_acc,
            sem_small, sem_bulk, sem_bulk2, sem_rest):

    def wq_block(j):
        slot = j & (SLOTS - 1)
        rows, left, right = pl.ds(_hint(j * 8, 8), 8), pl.ds(0, H * DH // 2), pl.ds(H * DH // 2, H * DH // 2)
        small = [(wq_hbm.at[i, rows, left], wq.at[i, rows, left], sem_small.at[slot]) for i in range(8)]
        return small, [(wq_hbm.at[:, rows, right], wq.at[:, rows, right], sem_bulk.at[slot])]

    def ffn_block(j):
        slot = j & (SLOTS - 1)

        def part(src, dst, first, count, sem):
            rows = pl.ds(_hint(j * FFN_ROWS + first, 32), count)
            return src.at[rows], dst.at[rows], sem.at[slot]

        small = []
        for u in range(5):
            small.append(part(wg_hbm, wg, 32 * u, 32, sem_small))
            if u < 3:
                small.append(part(wd_hbm, wd, 32 * u, 32, sem_small))
        return small, [part(wu_hbm, wu, 0, FFN_ROWS, sem_bulk), part(wd_hbm, wd, 96, FFN_ROWS - 96, sem_bulk)]

    def kv_block(n):
        slot = n & (SLOTS - 1)
        head = _hint((n // KEY_BLOCKS if isinstance(n, int) else lax.div(n, KEY_BLOCKS)) * G, G)
        keys = pl.ds(_hint((n & (KEY_BLOCKS - 1)) * T, T), T)
        small = [(k_hbm.at[head + i, keys], k_buf.at[slot, i], sem_small.at[slot]) for i in (0, 2, 4, 6, 1, 3, 5, 7)]
        return small, [(v_hbm.at[pl.ds(head, G), keys], v_buf.at[n & (V_SLOTS - 1)], sem_bulk.at[slot])]

    def wo_block(j):
        slot = j & (SLOTS - 1)

        def part(which, first, count, sem):
            rows = pl.ds(_hint(j * DH + first, 32), count)
            return wo_hbm.at[which, rows], wo.at[which, rows], sem.at[slot]

        small = [part(i % 4, 32 * (i // 4), 32, sem_small) for i in range(8)]
        return small, [part(pl.ds(0, 2), 64, 64, sem_bulk), part(pl.ds(2, 2), 64, 64, sem_bulk2)]

    last = pl.ds(W_BLOCKS * FFN_ROWS, F - W_BLOCKS * FFN_ROWS)
    rest = [(x_hbm, x_ref, sem_rest), (gw_hbm, gw_ref, sem_rest)] + [
        (src.at[last], dst.at[last], sem_rest) for src, dst in ((wg_hbm, wg), (wu_hbm, wu), (wd_hbm, wd))]

    def start(copies, priority):
        for c in copies:
            pltpu.make_async_copy(*c).start(priority=priority)

    def wait(copies):
        for c in copies:
            pltpu.make_async_copy(*c).wait()

    def wait_block(block):
        wait(block[1] + block[0])

    def wait_kv(n):
        slot = n & (SLOTS - 1)
        wait(kv_block(n)[1] + [(k_buf.at[slot], k_buf.at[slot], sem_small.at[slot])])

    def phase(count, stop, block, arrived, following, compute, carry):
        def body(ahead):
            def step(j, carry):
                arrived(j)
                if ahead is None:
                    return compute(j, carry)
                small, bulk = ahead(j + DEPTH)
                start(small[:1], 0)
                start(bulk, 1)
                carry = compute(j, carry)
                for c in small[1:]:
                    start([c], 0)
                    pl.delay(PAUSE_NS)
                return carry
            return step

        carry = lax.fori_loop(0, count - DEPTH, body(block), carry)
        return lax.fori_loop(count - DEPTH, stop, body(following and (lambda u: following(u - count))), carry)

    for j in range(DEPTH):
        start(wq_block(j)[1], 1)
    start(rest, 1)

    @pl.loop(0, DEPTH)
    def _(j):
        for c in wq_block(j)[0]:
            start([c], 0)
            pl.delay(FIRST_PAUSE_NS)

    for w in (wg, wu, wd):
        w[pl.ds(F, FFN_BANDS * DH - F), :] = jnp.zeros((FFN_BANDS * DH - F, D), BF16)
    v_buf[V_SLOTS - 1] = jnp.zeros((G, T, DH), BF16)
    ffn_acc[...] = jnp.zeros((G, D), F32)

    def idle(j, carry):
        pl.delay(PAUSE_NS)
        return carry

    phase(W_BLOCKS, W_BLOCKS, wq_block, lambda j: wait_block(wq_block(j)), ffn_block, idle, None)
    wait(rest)

    def load_x():
        x = x_ref[...].astype(F32)
        return jnp.concatenate([x, x], axis=0).astype(BF16)

    def project_q(j, carry):
        w = wq[:, :, pl.ds(_hint(j * (4 * DH), 4 * DH), 4 * DH)].reshape(D, 4 * DH)
        q = _dot(load_x(), w)
        for i in range(4):
            q_all[:, pl.ds(4 * j + i, 1), :] = q[:B, i * DH:(i + 1) * DH].reshape(B, 1, DH)
        return carry

    phase(W_BLOCKS, W_BLOCKS, ffn_block, lambda j: wait_block(ffn_block(j)), kv_block, project_q, None)

    row = lax.broadcasted_iota(jnp.int32, (G, DH), 0)

    def heads(g):
        return lax.div(g, H // G), pl.ds(_hint((g & (H // G - 1)) * G, G), G)

    def per_head(product):
        out = product(0)
        for i in range(1, G):
            out = jnp.where(row == i, product(i), out)
        return out

    def accumulate(n, m, total, acc, s):
        m_new = jnp.maximum(m, jnp.max(s, axis=1, keepdims=True))
        alpha = jnp.exp2((m - m_new) * EXP2_SCALE)
        e = jnp.exp2((s - m_new) * EXP2_SCALE)
        p = e.astype(BF16)
        pv = per_head(lambda i: _dot(p, v_buf[n & (V_SLOTS - 1), i]))
        return m_new, total * alpha + e, acc * alpha + pv

    def finish_group(g, total, acc):
        o_all[heads(g)] = acc / jnp.sum(total, axis=1, keepdims=True)

    def ffn_band(j):
        rows = pl.ds(_hint(j * DH, DH), DH)
        x = load_x()
        gate, up = _dot_nt(x, wg[rows, :]), _dot_nt(x, wu[rows, :])
        hidden = (gate * jax.nn.sigmoid(gate) * up).astype(BF16)
        ffn_acc[...] += _dot(hidden, wd[rows, :])

    def attend(n, carry):
        m, total, acc, s_prev = carry
        g, kb = lax.div(n, KEY_BLOCKS), n & (KEY_BLOCKS - 1)
        m, total, acc = accumulate(n + V_SLOTS - 1, m, total, acc, s_prev)
        q = q_all[heads(g)].astype(BF16)
        s = per_head(lambda i: _dot_nt(q, k_buf[n & (SLOTS - 1), i]))
        pl.when((kb == 0) & (n > 0))(lambda: finish_group(g - 1, total, acc))
        pl.when((kb == KEY_BLOCKS // 2) & (g < FFN_BANDS))(lambda: ffn_band(g))
        fresh = kb == 0
        return jnp.where(fresh, -jnp.inf, m), jnp.where(fresh, 0.0, total), jnp.where(fresh, 0.0, acc), s

    zero = ffn_acc[:, :DH]
    m, total, acc, s = phase(KV_BLOCKS, KV_BLOCKS, kv_block, wait_kv, wo_block, attend, (zero,) * 4)
    _, total, acc = accumulate(KV_BLOCKS - 1, m, total, acc, s)
    finish_group(jnp.int32(GROUPS - 1), total, acc)

    x, gw = x_ref[...].astype(F32), gw_ref[...].astype(F32)
    logit = sum(x[:, r * DH:(r + 1) * DH] * gw[r:r + 1, :] for r in range(D // DH))
    mix = jax.nn.sigmoid(jnp.sum(logit, axis=1, keepdims=True))

    def project_out(j, out, which=range(4)):
        rows = pl.ds(_hint(j * DH, DH), DH)
        attn = sum(_dot(o_all[:, pl.ds(8 * i + j, 1), :].reshape(B, DH).astype(BF16), wo[i, rows, :]) for i in which)
        return out + mix * attn

    out = (1.0 - mix) * ffn_acc[:B, :]
    out = phase(W_BLOCKS, W_BLOCKS - 1, wo_block, lambda j: wait_block(wo_block(j)), None, project_out, out)
    small, bulk = wo_block(W_BLOCKS - 1)
    wait(small + bulk[:1])
    out = project_out(W_BLOCKS - 1, out, (0, 1))
    wait(bulk[1:])
    o_ref[...] = project_out(W_BLOCKS - 1, out, (2, 3)).astype(o_ref.dtype)


@jax.jit
def pallas_gated_mix__mha_block_cached__swiglu_ffn__decode_kernel(
    A_x: jax.Array,
    A_k_cache: jax.Array,
    A_v_cache: jax.Array,
    A_wq: jax.Array,
    A_wo: jax.Array,
    B_x: jax.Array,
    B_w_gate: jax.Array,
    B_w_up: jax.Array,
    B_w_down: jax.Array,
    gate_w: jax.Array,
):
    del B_x
    hbm = pl.BlockSpec(memory_space=pltpu.HBM)
    out = pl.pallas_call(
        _kernel,
        name="gated_mix_decode",
        out_shape=jax.ShapeDtypeStruct((B, D), A_x.dtype),
        in_specs=[hbm] * 9,
        out_specs=pl.BlockSpec(memory_space=pltpu.VMEM),
        scratch_shapes=[
            pltpu.VMEM((SLOTS, G, T, DH), BF16),
            pltpu.VMEM((V_SLOTS, G, T, DH), BF16),
            pltpu.VMEM((8, D // 8, H * DH), BF16),
            pltpu.VMEM((4, H * DH // 4, D), BF16),
            pltpu.VMEM((FFN_BANDS * DH, D), BF16),
            pltpu.VMEM((FFN_BANDS * DH, D), BF16),
            pltpu.VMEM((FFN_BANDS * DH, D), BF16),
            pltpu.VMEM((B, D), BF16),
            pltpu.VMEM((D // DH, DH), BF16),
            pltpu.VMEM((B, H, DH), F32),
            pltpu.VMEM((B, H, DH), F32),
            pltpu.VMEM((G, D), F32),
            pltpu.SemaphoreType.DMA((SLOTS,)),
            pltpu.SemaphoreType.DMA((SLOTS,)),
            pltpu.SemaphoreType.DMA((SLOTS,)),
            pltpu.SemaphoreType.DMA,
        ],
        compiler_params=pltpu.CompilerParams(
            vmem_limit_bytes=40 * 1024 * 1024,
            disable_semaphore_checks=True,
        ),
    )(
        A_x.reshape(B, D),
        A_k_cache.reshape(B * H, SK, DH),
        A_v_cache.reshape(B * H, SK, DH),
        A_wq.reshape(8, D // 8, H * DH),
        A_wo.reshape(4, H * DH // 4, D),
        B_w_gate.T,
        B_w_up.T,
        B_w_down,
        gate_w.reshape(D // DH, DH),
    )
    return out.reshape(B, 1, D)
```

```python
import math

import jax
import jax.numpy as jnp
from jax import lax
from jax.experimental import pallas as pl
from jax.experimental.pallas import tpu as pltpu

B, D, H, SK, DH, F = 4, 512, 32, 4096, 128, 1376

T = 128
G = 8
KEY_BLOCKS = SK // T
GROUPS = B * H // G
KV_BLOCKS = GROUPS * KEY_BLOCKS
W_BLOCKS = 8
FFN_ROWS = 160
FFN_BANDS = -(-F // DH)

DEPTH = 3
SLOTS = 4
V_SLOTS = 8
K_ORDER = (7, 0, 2, 4, 6, 1, 3, 5)
KV_PAUSE = (12, 12, 10, 10, 10, 10)
W_PAUSE = (9,) * 6
IDLE_PAUSE = (13,) * 6

EXP2_SCALE = DH ** -0.5 * math.log2(math.e)
F32, BF16 = jnp.float32, jnp.bfloat16


def _hint(v, m):
    return v if isinstance(v, int) else pl.multiple_of(v, m)


def _dot(a, b):
    return jnp.dot(a, b, preferred_element_type=F32)


def _dot_nt(a, b):
    return lax.dot_general(a, b, (((1,), (1,)), ((), ())), preferred_element_type=F32)


def _start(copies, priority):
    for c in copies:
        pltpu.make_async_copy(*c).start(priority=priority)


def _wait(copies):
    for c in copies:
        pltpu.make_async_copy(*c).wait()


def _pause(tick, steps):
    return lax.fori_loop(0, steps, lambda _, t: (t * 3 + 1) & 0xFFFF, tick)


def _phase(count, stop, block, following, compute, pauses, tick, carry):
    def body(ahead):
        def step(j, state):
            tick, carry = state
            small, bulk = block(j)
            _wait(bulk + small)
            if ahead is None:
                return tick, compute(j, carry)
            small, bulk = ahead(j + DEPTH)
            _start(small[:1], 0)
            _start(bulk, 1)
            carry = compute(j, carry)
            _start(small[1:2], 0)
            for c, steps in zip(small[2:], pauses, strict=True):
                tick = _pause(tick, steps)
                _start([c], 0)
            return tick, carry
        return step

    state = lax.fori_loop(0, count - DEPTH, body(block), (tick, carry))
    return lax.fori_loop(count - DEPTH, stop, body(following and (lambda u: following(u - count))), state)


def _kernel(x_hbm, k_hbm, v_hbm, wq_hbm, wo_hbm, wg_hbm, wu_hbm, wd_hbm, gw_hbm, o_ref,
            k_buf, v_buf, wq, wo, wg, wu, wd, x_ref, gw_ref, q_all, o_all, ffn_acc, tick_ref, sem_aside):

    def project_out(j, out, mix, which):
        rows = pl.ds(_hint(j * DH, DH), DH)
        attn = sum(_dot(o_all[:, pl.ds(8 * i + j, 1), :].reshape(B, DH).astype(BF16), wo[i, rows, :]) for i in which)
        return out + mix * attn

    def wo_part(j, which, first, count, sem):
        rows = pl.ds(_hint(j * DH + first, 32), count)
        return wo_hbm.at[which, rows], wo.at[which, rows], sem

    def stream(sem_small, sem_bulk):
        def wq_block(j):
            slot, half = j & (SLOTS - 1), H * DH // 2
            rows, left, right = pl.ds(_hint(j * 8, 8), 8), pl.ds(0, half), pl.ds(half, half)
            small = [(wq_hbm.at[i, rows, left], wq.at[i, rows, left], sem_small.at[slot]) for i in range(8)]
            return small, [(wq_hbm.at[:, rows, right], wq.at[:, rows, right], sem_bulk.at[slot])]

        def ffn_block(j):
            slot = j & (SLOTS - 1)

            def part(src, dst, first, count, sem):
                rows = pl.ds(_hint(j * FFN_ROWS + first, 32), count)
                return src.at[rows], dst.at[rows], sem.at[slot]

            small = []
            for u in range(5):
                small.append(part(wg_hbm, wg, 32 * u, 32, sem_small))
                if u < 3:
                    small.append(part(wd_hbm, wd, 32 * u, 32, sem_small))
            return small, [part(wu_hbm, wu, 0, FFN_ROWS, sem_bulk), part(wd_hbm, wd, 96, FFN_ROWS - 96, sem_bulk)]

        def kv_block(n):
            slot, g = n & (SLOTS - 1), lax.div(n, KEY_BLOCKS)
            keys = pl.ds(_hint((n & (KEY_BLOCKS - 1)) * T, T), T)
            pairs = pl.ds(_hint(g * (G // 2), G // 2), G // 2)
            small = [(k_hbm.at[g * G + i, keys], k_buf.at[slot, i], sem_small.at[slot]) for i in K_ORDER]
            return small, [(v_hbm.at[pairs, u, keys], v_buf.at[n & (V_SLOTS - 1), :, u], sem_bulk.at[slot])
                           for u in range(2)]

        def wo_block(j):
            slot = j & (SLOTS - 1)
            small = [wo_part(j, i % 4, 32 * (i // 4), 32, sem_small.at[slot]) for i in range(8)]
            return small, [wo_part(j, pl.ds(i, 2), 64, 64, sem_bulk.at[slot]) for i in (0, 2)]

        last = pl.ds(W_BLOCKS * FFN_ROWS, F - W_BLOCKS * FFN_ROWS)
        rest = [(x_hbm, x_ref, sem_aside), (gw_hbm, gw_ref, sem_aside)] + [
            (src.at[last], dst.at[last], sem_aside) for src, dst in ((wg_hbm, wg), (wu_hbm, wu), (wd_hbm, wd))]

        for j in range(DEPTH):
            _start(wq_block(j)[1], 1)
        _start(rest, 1)

        def fill(j, tick):
            for c in wq_block(j)[0]:
                _start([c], 0)
                tick = _pause(tick, IDLE_PAUSE[0])
            return tick

        tick = lax.fori_loop(0, DEPTH, fill, jnp.int32(0))

        for w in (wg, wu, wd):
            w[pl.ds(F, FFN_BANDS * DH - F), :] = jnp.zeros((FFN_BANDS * DH - F, D), BF16)
        v_buf[V_SLOTS - 1] = jnp.zeros(v_buf.shape[1:], BF16)
        ffn_acc[...] = jnp.zeros((G, D), F32)

        tick, idle = _phase(W_BLOCKS, W_BLOCKS, wq_block, ffn_block,
                            lambda j, t: _pause(t, IDLE_PAUSE[0]), IDLE_PAUSE, tick, tick)
        _wait(rest)

        def load_x():
            x = x_ref[...].astype(F32)
            return jnp.concatenate([x, x], axis=0).astype(BF16)

        def project_q(j, carry):
            w = wq[:, :, pl.ds(_hint(j * (4 * DH), 4 * DH), 4 * DH)].reshape(D, 4 * DH)
            q = _dot(load_x(), w)
            for i in range(4):
                q_all[:, pl.ds(4 * j + i, 1), :] = q[:B, i * DH:(i + 1) * DH].reshape(B, 1, DH)
            return carry

        tick, _ = _phase(W_BLOCKS, W_BLOCKS, ffn_block, kv_block, project_q, W_PAUSE, tick + idle, None)

        row = lax.broadcasted_iota(jnp.int32, (G, DH), 0)

        def heads(g):
            return lax.div(g, H // G), pl.ds(_hint((g & (H // G - 1)) * G, G), G)

        def per_head(product):
            out = product(0)
            for i in range(1, G):
                out = jnp.where(row == i, product(i), out)
            return out

        def accumulate(n, m, total, acc, s):
            m_new = jnp.maximum(m, jnp.max(s, axis=1, keepdims=True))
            alpha = jnp.exp2((m - m_new) * EXP2_SCALE)
            e = jnp.exp2((s - m_new) * EXP2_SCALE)
            p = e.astype(BF16)
            pv = per_head(lambda i: _dot(p, v_buf[n & (V_SLOTS - 1), i // 2, i % 2]))
            return m_new, total * alpha + e, acc * alpha + pv

        def finish_group(g, total, acc):
            o_all[heads(g)] = acc / jnp.sum(total, axis=1, keepdims=True)

        def ffn_band(j):
            rows = pl.ds(_hint(j * DH, DH), DH)
            x = load_x()
            gate, up = _dot_nt(x, wg[rows, :]), _dot_nt(x, wu[rows, :])
            hidden = (gate * jax.nn.sigmoid(gate) * up).astype(BF16)
            ffn_acc[...] += _dot(hidden, wd[rows, :])

        def attend(n, carry):
            m, total, acc, s_prev = carry
            g, kb = lax.div(n, KEY_BLOCKS), n & (KEY_BLOCKS - 1)
            m, total, acc = accumulate(n + V_SLOTS - 1, m, total, acc, s_prev)
            q = q_all[heads(g)].astype(BF16)
            s = per_head(lambda i: _dot_nt(q, k_buf[n & (SLOTS - 1), i]))
            pl.when((kb == 0) & (n > 0))(lambda: finish_group(g - 1, total, acc))
            pl.when((kb == KEY_BLOCKS // 2) & (g < FFN_BANDS))(lambda: ffn_band(g))
            fresh = kb == 0
            return jnp.where(fresh, -jnp.inf, m), jnp.where(fresh, 0.0, total), jnp.where(fresh, 0.0, acc), s

        zero = ffn_acc[:, :DH]
        tick, (m, total, acc, s) = _phase(KV_BLOCKS, KV_BLOCKS, kv_block, wo_block, attend, KV_PAUSE, tick, (zero,) * 4)
        _, total, acc = accumulate(KV_BLOCKS - 1, m, total, acc, s)
        finish_group(jnp.int32(GROUPS - 1), total, acc)

        x, gw = x_ref[...].astype(F32), gw_ref[...].astype(F32)
        logit = sum(x[:, r * DH:(r + 1) * DH] * gw[r:r + 1, :] for r in range(D // DH))
        mix = jax.nn.sigmoid(jnp.sum(logit, axis=1, keepdims=True))

        def final_block(_):
            small, bulk = wo_block(W_BLOCKS - 1)
            return small, [bulk[0], wo_part(W_BLOCKS - 1, pl.ds(2, 2), 64, 64, sem_aside)]

        out = (1.0 - mix) * ffn_acc[:B, :]
        project = lambda j, out: project_out(j, out, mix, range(4))
        tick, out = _phase(W_BLOCKS - 1, W_BLOCKS - DEPTH, wo_block, final_block, project, W_PAUSE, tick, out)
        tick_ref[0] = tick

        def drain(j, out):
            _wait(sum(wo_block(j), []))
            return project(j, out)

        out = lax.fori_loop(W_BLOCKS - DEPTH, W_BLOCKS - 1, drain, out)
        small, bulk = wo_block(W_BLOCKS - 1)
        _wait(small + bulk[:1])
        return project_out(W_BLOCKS - 1, out, mix, (0, 1)), mix

    out, mix = pl.run_scoped(stream, pltpu.SemaphoreType.DMA((SLOTS,)), pltpu.SemaphoreType.DMA((SLOTS,)))
    _wait([wo_part(W_BLOCKS - 1, pl.ds(2, 2), 64, 64, sem_aside)])
    o_ref[...] = project_out(W_BLOCKS - 1, out, mix, (2, 3)).astype(o_ref.dtype)


@jax.jit
def pallas_gated_mix__mha_block_cached__swiglu_ffn__decode_kernel(
    A_x: jax.Array,
    A_k_cache: jax.Array,
    A_v_cache: jax.Array,
    A_wq: jax.Array,
    A_wo: jax.Array,
    B_x: jax.Array,
    B_w_gate: jax.Array,
    B_w_up: jax.Array,
    B_w_down: jax.Array,
    gate_w: jax.Array,
):
    del B_x
    hbm = pl.BlockSpec(memory_space=pltpu.HBM)
    out = pl.pallas_call(
        _kernel,
        name="gated_mix_decode",
        out_shape=jax.ShapeDtypeStruct((B, D), A_x.dtype),
        in_specs=[hbm] * 9,
        out_specs=pl.BlockSpec(memory_space=pltpu.VMEM),
        scratch_shapes=[
            pltpu.VMEM((SLOTS, G, T, DH), BF16),
            pltpu.VMEM((V_SLOTS, G // 2, 2, T, DH), BF16),
            pltpu.VMEM((8, D // 8, H * DH), BF16),
            pltpu.VMEM((4, H * DH // 4, D), BF16),
            pltpu.VMEM((FFN_BANDS * DH, D), BF16),
            pltpu.VMEM((FFN_BANDS * DH, D), BF16),
            pltpu.VMEM((FFN_BANDS * DH, D), BF16),
            pltpu.VMEM((B, D), BF16),
            pltpu.VMEM((D // DH, DH), BF16),
            pltpu.VMEM((B, H, DH), F32),
            pltpu.VMEM((B, H, DH), F32),
            pltpu.VMEM((G, D), F32),
            pltpu.SMEM((1,), jnp.int32),
            pltpu.SemaphoreType.DMA,
        ],
        compiler_params=pltpu.CompilerParams(
            vmem_limit_bytes=40 * 1024 * 1024,
        ),
    )(
        A_x.reshape(B, D),
        A_k_cache.reshape(B * H, SK, DH),
        A_v_cache.reshape(B * H // 2, 2, SK, DH),
        A_wq.reshape(8, D // 8, H * DH),
        A_wo.reshape(4, H * DH // 4, D),
        B_w_gate.T,
        B_w_up.T,
        B_w_down,
        gate_w.reshape(D // DH, DH),
    )
    return out.reshape(B, 1, D)
```

```python
import functools
import math

import jax
import jax.numpy as jnp
from jax import lax
from jax.experimental import pallas as pl
from jax.experimental.pallas import tpu as pltpu

B, D, H, SK, DH, F = 4, 512, 32, 4096, 128, 1376

T = 128
G = 8
KEY_BLOCKS = SK // T
GROUPS = B * H // G
KV_BLOCKS = GROUPS * KEY_BLOCKS
W_BLOCKS = 8
FFN_ROWS = 160
FFN_BANDS = -(-F // DH)

DEPTH = 3
SLOTS = 4
V_SLOTS = 8
K_ORDER = (7, 0, 2, 4, 6, 1, 3, 5)
PAUSE = 10
IDLE_PAUSE = 14

EXP2_SCALE = DH ** -0.5 * math.log2(math.e)
F32, BF16 = jnp.float32, jnp.bfloat16


def _hint(v, m):
    return v if isinstance(v, int) else pl.multiple_of(v, m)


def _dot(a, b):
    return jnp.dot(a, b, preferred_element_type=F32)


def _dot_nt(a, b):
    return lax.dot_general(a, b, (((1,), (1,)), ((), ())), preferred_element_type=F32)


def _start(copies, priority):
    for c in copies:
        pltpu.make_async_copy(*c).start(priority=priority)


def _wait(copies):
    for c in copies:
        pltpu.make_async_copy(*c).wait()


def _stream(x_hbm, k_hbm, v_hbm, wq_hbm, wo_hbm, wg_hbm, wu_hbm, wd_hbm, gw_hbm, o_ref,
            k_buf, v_buf, wq, wo, wg, wu, wd, x_ref, gw_ref, q_all, o_all, ffn_acc, tick_ref,
            sem_small, sem_bulk):

    def wq_block(j):
        def part(which, half, sem):
            at = (which, pl.ds(_hint(j * 8, 8), 8), pl.ds(half * (H * DH // 2), H * DH // 2))
            return wq_hbm.at[at], wq.at[at], sem.at[j & (SLOTS - 1)]

        small = [part(i % 4, i // 4, sem_small) for i in range(8)]
        return small, [part(pl.ds(4, 4), half, sem_bulk) for half in range(2)]

    def ffn_block(j):
        def part(src, dst, first, count, sem):
            rows = pl.ds(_hint(j * FFN_ROWS + first, 32), count)
            return src.at[rows], dst.at[rows], sem.at[j & (SLOTS - 1)]

        small = []
        for u in range(5):
            small.append(part(wg_hbm, wg, 32 * u, 32, sem_small))
            if u < 3:
                small.append(part(wd_hbm, wd, 32 * u, 32, sem_small))
        return small, [part(wu_hbm, wu, 0, FFN_ROWS, sem_bulk), part(wd_hbm, wd, 96, FFN_ROWS - 96, sem_bulk)]

    def kv_block(n):
        slot, g = n & (SLOTS - 1), lax.div(n, KEY_BLOCKS)
        keys = pl.ds(_hint((n & (KEY_BLOCKS - 1)) * T, T), T)
        pairs = pl.ds(_hint(g * (G // 2), G // 2), G // 2)
        small = [(k_hbm.at[g * G + i, keys], k_buf.at[slot, i], sem_small.at[slot]) for i in K_ORDER]
        bulk = [(v_hbm.at[pairs, u, keys], v_buf.at[n & (V_SLOTS - 1), :, u], sem_bulk.at[slot]) for u in range(2)]
        return small, bulk

    def wo_block(j):
        def part(which, u, sem):
            rows = pl.ds(_hint(j * DH + 32 * u, 32), 32)
            return wo_hbm.at[which, rows], wo.at[which, rows], sem.at[j & (SLOTS - 1)]

        small = [part(i % 2, i // 2, sem_small) for i in range(8)]
        return small, [part(pl.ds(2, 2), u, sem_bulk) for u in range(4)]

    last_rows = pl.ds(W_BLOCKS * FFN_ROWS, F - W_BLOCKS * FFN_ROWS)
    rest = [(x_hbm, x_ref), (gw_hbm, gw_ref)]
    rest += [(src.at[last_rows], dst.at[last_rows]) for src, dst in ((wg_hbm, wg), (wu_hbm, wu), (wd_hbm, wd))]
    rest = [(src, dst, sem_bulk.at[SLOTS]) for src, dst in rest]

    def pause(steps):
        tick_ref[0] = lax.fori_loop(0, steps, lambda _, t: (t * 3 + 1) & 0xFFFF, tick_ref[0])

    def consume(first, stop, block, ahead, compute, carry, steps=PAUSE):
        def step(j, carry):
            small, bulk = block(j)
            _wait(bulk + small)
            small, bulk = ahead(j + DEPTH)
            _start(small[:1], 0)
            _start(bulk, 1)
            carry = compute(j, carry)
            _start(small[1:2], 0)
            for c in small[2:]:
                pause(steps)
                _start([c], 0)
            return carry

        return lax.fori_loop(first, stop, step, carry)

    def phase(count, block, following, compute, carry, steps=PAUSE):
        carry = consume(0, count - DEPTH, block, block, compute, carry, steps)
        return consume(count - DEPTH, count, block, lambda u: following(u - count), compute, carry, steps)

    for j in range(DEPTH):
        _start(wq_block(j)[1], 1)
    _start(rest, 1)
    tick_ref[0] = 0

    @pl.loop(0, DEPTH)
    def _(j):
        for c in wq_block(j)[0]:
            _start([c], 0)
            pause(IDLE_PAUSE)

    for w in (wg, wu, wd):
        w[pl.ds(F, FFN_BANDS * DH - F), :] = jnp.zeros((FFN_BANDS * DH - F, D), BF16)
    v_buf[V_SLOTS - 1] = jnp.zeros(v_buf.shape[1:], BF16)
    ffn_acc[...] = jnp.zeros((G, D), F32)

    phase(W_BLOCKS, wq_block, ffn_block, lambda j, _: pause(IDLE_PAUSE), None, IDLE_PAUSE)
    _wait(rest)

    def load_x():
        x = x_ref[...].astype(F32)
        return jnp.concatenate([x, x], axis=0).astype(BF16)

    def project_q(j, _):
        w = wq[:, :, pl.ds(_hint(j * (4 * DH), 4 * DH), 4 * DH)].reshape(D, 4 * DH)
        q = _dot(load_x(), w)
        for i in range(4):
            q_all[:, pl.ds(4 * j + i, 1), :] = q[:B, i * DH:(i + 1) * DH].reshape(B, 1, DH)

    phase(W_BLOCKS, ffn_block, kv_block, project_q, None)

    row = lax.broadcasted_iota(jnp.int32, (G, DH), 0)

    def heads(g):
        return lax.div(g, H // G), pl.ds(_hint((g & (H // G - 1)) * G, G), G)

    def per_head(product):
        out = product(0)
        for i in range(1, G):
            out = jnp.where(row == i, product(i), out)
        return out

    def accumulate(n, m, total, acc, s):
        m_new = jnp.maximum(m, jnp.max(s, axis=1, keepdims=True))
        alpha = jnp.exp2((m - m_new) * EXP2_SCALE)
        e = jnp.exp2((s - m_new) * EXP2_SCALE)
        p = e.astype(BF16)
        pv = per_head(lambda i: _dot(p, v_buf[n & (V_SLOTS - 1), i // 2, i % 2]))
        return m_new, total * alpha + e, acc * alpha + pv

    def finish_group(g, total, acc):
        o_all[heads(g)] = acc / jnp.sum(total, axis=1, keepdims=True)

    def ffn_band(j):
        rows = pl.ds(_hint(j * DH, DH), DH)
        x = load_x()
        gate, up = _dot_nt(x, wg[rows, :]), _dot_nt(x, wu[rows, :])
        hidden = (gate * jax.nn.sigmoid(gate) * up).astype(BF16)
        ffn_acc[...] += _dot(hidden, wd[rows, :])

    def attend(n, carry):
        m, total, acc, s_prev = carry
        g, kb = lax.div(n, KEY_BLOCKS), n & (KEY_BLOCKS - 1)
        m, total, acc = accumulate(n + V_SLOTS - 1, m, total, acc, s_prev)
        q = q_all[heads(g)].astype(BF16)
        s = per_head(lambda i: _dot_nt(q, k_buf[n & (SLOTS - 1), i]))
        pl.when((kb == 0) & (n > 0))(lambda: finish_group(g - 1, total, acc))
        pl.when((kb == KEY_BLOCKS // 2) & (g < FFN_BANDS))(lambda: ffn_band(g))
        fresh = kb == 0
        return jnp.where(fresh, -jnp.inf, m), jnp.where(fresh, 0.0, total), jnp.where(fresh, 0.0, acc), s

    zero = ffn_acc[:, :DH]
    m, total, acc, s = phase(KV_BLOCKS, kv_block, wo_block, attend, (zero,) * 4)
    _, total, acc = accumulate(KV_BLOCKS - 1, m, total, acc, s)
    finish_group(jnp.int32(GROUPS - 1), total, acc)

    x, gw = x_ref[...].astype(F32), gw_ref[...].astype(F32)
    logit = sum(x[:, r * DH:(r + 1) * DH] * gw[r:r + 1, :] for r in range(D // DH))
    mix = jax.nn.sigmoid(jnp.sum(logit, axis=1, keepdims=True))

    def project_out(j, out, which=(0, 1, 2, 3)):
        rows = pl.ds(_hint(j * DH, DH), DH)
        attn = sum(_dot(o_all[:, pl.ds(8 * i + j, 1), :].reshape(B, DH).astype(BF16), wo[i, rows, :]) for i in which)
        return out + mix * attn

    out = (1.0 - mix) * ffn_acc[:B, :]
    out = consume(0, W_BLOCKS - DEPTH, wo_block, wo_block, project_out, out)

    def early(j, out):
        _wait(wo_block(j)[0])
        return project_out(j, out, (0, 1))

    def late(j, out):
        _wait(wo_block(j)[1])
        return project_out(j, out, (2, 3))

    out = late(W_BLOCKS - DEPTH, out)
    out = lax.fori_loop(W_BLOCKS - DEPTH, W_BLOCKS, early, out)
    out = lax.fori_loop(W_BLOCKS - DEPTH + 1, W_BLOCKS, late, out)
    o_ref[...] = out.astype(o_ref.dtype)


def _kernel(*refs):
    pl.run_scoped(functools.partial(_stream, *refs),
                  pltpu.SemaphoreType.DMA((SLOTS,)), pltpu.SemaphoreType.DMA((SLOTS + 1,)))


@jax.jit
def pallas_gated_mix__mha_block_cached__swiglu_ffn__decode_kernel(
    A_x: jax.Array,
    A_k_cache: jax.Array,
    A_v_cache: jax.Array,
    A_wq: jax.Array,
    A_wo: jax.Array,
    B_x: jax.Array,
    B_w_gate: jax.Array,
    B_w_up: jax.Array,
    B_w_down: jax.Array,
    gate_w: jax.Array,
):
    del B_x
    hbm = pl.BlockSpec(memory_space=pltpu.HBM)
    out = pl.pallas_call(
        _kernel,
        name="gated_mix_decode",
        out_shape=jax.ShapeDtypeStruct((B, D), A_x.dtype),
        in_specs=[hbm] * 9,
        out_specs=pl.BlockSpec(memory_space=pltpu.VMEM),
        scratch_shapes=[
            pltpu.VMEM((SLOTS, G, T, DH), BF16),
            pltpu.VMEM((V_SLOTS, G // 2, 2, T, DH), BF16),
            pltpu.VMEM((8, D // 8, H * DH), BF16),
            pltpu.VMEM((4, H * DH // 4, D), BF16),
            pltpu.VMEM((FFN_BANDS * DH, D), BF16),
            pltpu.VMEM((FFN_BANDS * DH, D), BF16),
            pltpu.VMEM((FFN_BANDS * DH, D), BF16),
            pltpu.VMEM((B, D), BF16),
            pltpu.VMEM((D // DH, DH), BF16),
            pltpu.VMEM((B, H, DH), F32),
            pltpu.VMEM((B, H, DH), F32),
            pltpu.VMEM((G, D), F32),
            pltpu.SMEM((1,), jnp.int32),
        ],
        compiler_params=pltpu.CompilerParams(vmem_limit_bytes=40 * 1024 * 1024),
    )(
        A_x.reshape(B, D),
        A_k_cache.reshape(B * H, SK, DH),
        A_v_cache.reshape(B * H // 2, 2, SK, DH),
        A_wq.reshape(8, D // 8, H * DH),
        A_wo.reshape(4, H * DH // 4, D),
        B_w_gate.T,
        B_w_up.T,
        B_w_down,
        gate_w.reshape(D // DH, DH),
    )
    return out.reshape(B, 1, D)
```

```python
import functools
import math

import jax
import jax.numpy as jnp
from jax import lax
from jax.experimental import pallas as pl
from jax.experimental.pallas import tpu as pltpu

B, D, H, SK, DH, F = 4, 512, 32, 4096, 128, 1376

T = 128
G = 8
KEY_BLOCKS = SK // T
GROUPS = B * H // G
KV_BLOCKS = GROUPS * KEY_BLOCKS
W_BLOCKS = 8
FFN_ROWS = 160
FFN_BANDS = -(-F // DH)

DEPTH = 3
SLOTS = 4
V_SLOTS = 8
K_ORDER = (7, 0, 2, 4, 6, 1, 3, 5)
PAUSE = 10
IDLE_PAUSE = 14

EXP2_SCALE = DH ** -0.5 * math.log2(math.e)
F32, BF16 = jnp.float32, jnp.bfloat16


def _hint(v, m):
    return v if isinstance(v, int) else pl.multiple_of(v, m)


def _dot(a, b):
    return jnp.dot(a, b, preferred_element_type=F32)


def _dot_nt(a, b):
    return lax.dot_general(a, b, (((1,), (1,)), ((), ())), preferred_element_type=F32)


def _start(copies, priority):
    for c in copies:
        pltpu.make_async_copy(*c).start(priority=priority)


def _wait(copies):
    for c in copies:
        pltpu.make_async_copy(*c).wait()


def _stream(x_hbm, k_hbm, v_hbm, wq_hbm, wo_hbm, wg_hbm, wu_hbm, wd_hbm, gw_hbm, o_ref,
            k_buf, v_buf, wq, wo, wg, wu, wd, x_ref, gw_ref, q_all, o_all, ffn_acc, tick_ref,
            sem_small, sem_bulk):

    def wq_block(j):
        def part(which, half, sem):
            at = (which, pl.ds(_hint(j * 8, 8), 8), pl.ds(half * (H * DH // 2), H * DH // 2))
            return wq_hbm.at[at], wq.at[at], sem.at[j & (SLOTS - 1)]

        small = [part(i % 4, i // 4, sem_small) for i in range(8)]
        return small, [part(pl.ds(4, 4), half, sem_bulk) for half in range(2)]

    def ffn_block(j):
        def part(src, dst, first, count, sem):
            rows = pl.ds(_hint(j * FFN_ROWS + first, 32), count)
            return src.at[rows], dst.at[rows], sem.at[j & (SLOTS - 1)]

        small = []
        for u in range(5):
            small.append(part(wg_hbm, wg, 32 * u, 32, sem_small))
            if u < 3:
                small.append(part(wd_hbm, wd, 32 * u, 32, sem_small))
        return small, [part(wu_hbm, wu, 0, FFN_ROWS, sem_bulk), part(wd_hbm, wd, 96, FFN_ROWS - 96, sem_bulk)]

    def kv_block(n):
        slot, g = n & (SLOTS - 1), lax.div(n, KEY_BLOCKS)
        keys = pl.ds(_hint((n & (KEY_BLOCKS - 1)) * T, T), T)
        pairs = pl.ds(_hint(g * (G // 2), G // 2), G // 2)
        small = [(k_hbm.at[g * G + i, keys], k_buf.at[slot, i], sem_small.at[slot]) for i in K_ORDER]
        bulk = [(v_hbm.at[pairs, u, keys], v_buf.at[n & (V_SLOTS - 1), :, u], sem_bulk.at[slot]) for u in range(2)]
        return small, bulk

    def wo_block(j):
        def part(which, u, sem):
            rows = pl.ds(_hint(j * DH + 32 * u, 32), 32)
            return wo_hbm.at[which, rows], wo.at[which, rows], sem.at[j & (SLOTS - 1)]

        small = [part(i % 2, i // 2, sem_small) for i in range(8)]
        return small, [part(pl.ds(2, 2), u, sem_bulk) for u in range(4)]

    last_rows = pl.ds(W_BLOCKS * FFN_ROWS, F - W_BLOCKS * FFN_ROWS)
    rest = [(x_hbm, x_ref), (gw_hbm, gw_ref)]
    rest += [(src.at[last_rows], dst.at[last_rows]) for src, dst in ((wg_hbm, wg), (wu_hbm, wu), (wd_hbm, wd))]
    rest = [(src, dst, sem_bulk.at[SLOTS]) for src, dst in rest]

    def start_spaced(copies, steps, tick):
        _start(copies[:1], 0)
        for c in copies[1:]:
            tick = lax.fori_loop(0, steps, lambda _, t: (t * 3 + 1) & 0xFFFF, tick)
            _start([c], 0)
        tick_ref[0] = tick

    def wait_block(block, j):
        small, bulk = block(j)
        if block is kv_block:
            slot = j & (SLOTS - 1)
            small = [(k_buf.at[slot], k_buf.at[slot], sem_small.at[slot])]
        _wait(bulk + small)

    def consume(first, stop, block, ahead, compute, carry):
        def step(j, carry):
            wait_block(block, j)
            small, bulk = ahead(j + DEPTH)
            if compute is None:
                _start(bulk, 1)
                return start_spaced(small, IDLE_PAUSE, j)
            _start(small[:1], 0)
            _start(bulk, 1)
            carry = compute(j, carry)
            start_spaced(small[1:], PAUSE, j)
            return carry

        return lax.fori_loop(first, stop, step, carry)

    def phase(count, block, following, compute, carry):
        carry = consume(0, count - DEPTH, block, block, compute, carry)
        return consume(count - DEPTH, count, block, lambda u: following(u - count), compute, carry)

    for j in range(DEPTH):
        _start(wq_block(j)[1], 1)
    _start(rest, 1)

    start_spaced(sum((wq_block(j)[0] for j in range(DEPTH)), []), IDLE_PAUSE, jnp.int32(0))

    for w in (wg, wu, wd):
        w[pl.ds(F, FFN_BANDS * DH - F), :] = jnp.zeros((FFN_BANDS * DH - F, D), BF16)
    v_buf[V_SLOTS - 1] = jnp.zeros(v_buf.shape[1:], BF16)
    ffn_acc[...] = jnp.zeros((G, D), F32)

    phase(W_BLOCKS, wq_block, ffn_block, None, None)
    _wait(rest)

    def load_x():
        x = x_ref[...].astype(F32)
        return jnp.concatenate([x, x], axis=0).astype(BF16)

    def project_q(j, _):
        w = wq[:, :, pl.ds(_hint(j * (4 * DH), 4 * DH), 4 * DH)].reshape(D, 4 * DH)
        q = _dot(load_x(), w)
        for i in range(4):
            q_all[:, pl.ds(4 * j + i, 1), :] = q[:B, i * DH:(i + 1) * DH].reshape(B, 1, DH)

    phase(W_BLOCKS, ffn_block, kv_block, project_q, None)

    row = lax.broadcasted_iota(jnp.int32, (G, DH), 0)

    def heads(g):
        return lax.div(g, H // G), pl.ds(_hint((g & (H // G - 1)) * G, G), G)

    def per_head(product):
        out = product(0)
        for i in range(1, G):
            out = jnp.where(row == i, product(i), out)
        return out

    def accumulate(n, m, total, acc, s):
        m_new = jnp.maximum(m, jnp.max(s, axis=1, keepdims=True))
        alpha = jnp.exp2((m - m_new) * EXP2_SCALE)
        e = jnp.exp2((s - m_new) * EXP2_SCALE)
        p = e.astype(BF16)
        pv = per_head(lambda i: _dot(p, v_buf[n & (V_SLOTS - 1), i // 2, i % 2]))
        return m_new, total * alpha + e, acc * alpha + pv

    def finish_group(g, total, acc):
        o_all[heads(g)] = acc / jnp.sum(total, axis=1, keepdims=True)

    def ffn_band(j):
        rows = pl.ds(_hint(j * DH, DH), DH)
        x = load_x()
        gate, up = _dot_nt(x, wg[rows, :]), _dot_nt(x, wu[rows, :])
        hidden = (gate * jax.nn.sigmoid(gate) * up).astype(BF16)
        ffn_acc[...] += _dot(hidden, wd[rows, :])

    def attend(n, carry):
        m, total, acc, s_prev = carry
        g, kb = lax.div(n, KEY_BLOCKS), n & (KEY_BLOCKS - 1)
        m, total, acc = accumulate(n + V_SLOTS - 1, m, total, acc, s_prev)
        q = q_all[heads(g)].astype(BF16)
        s = per_head(lambda i: _dot_nt(q, k_buf[n & (SLOTS - 1), i]))
        pl.when((kb == 0) & (n > 0))(lambda: finish_group(g - 1, total, acc))
        pl.when((kb == KEY_BLOCKS // 2) & (g < FFN_BANDS))(lambda: ffn_band(g))
        fresh = kb == 0
        return jnp.where(fresh, -jnp.inf, m), jnp.where(fresh, 0.0, total), jnp.where(fresh, 0.0, acc), s

    zero = ffn_acc[:, :DH]
    m, total, acc, s = phase(KV_BLOCKS, kv_block, wo_block, attend, (zero,) * 4)
    _, total, acc = accumulate(KV_BLOCKS - 1, m, total, acc, s)
    finish_group(jnp.int32(GROUPS - 1), total, acc)

    x, gw = x_ref[...].astype(F32), gw_ref[...].astype(F32)
    logit = sum(x[:, r * DH:(r + 1) * DH] * gw[r:r + 1, :] for r in range(D // DH))
    mix = jax.nn.sigmoid(jnp.sum(logit, axis=1, keepdims=True))

    def project_out(j, out, which=(0, 1, 2, 3)):
        rows = pl.ds(_hint(j * DH, DH), DH)
        attn = sum(_dot(o_all[:, pl.ds(8 * i + j, 1), :].reshape(B, DH).astype(BF16), wo[i, rows, :]) for i in which)
        return out + mix * attn

    out = (1.0 - mix) * ffn_acc[:B, :]
    out = consume(0, W_BLOCKS - DEPTH, wo_block, wo_block, project_out, out)

    def early(j, out):
        _wait(wo_block(j)[0])
        return project_out(j, out, (0, 1))

    def late(j, out):
        _wait(wo_block(j)[1])
        return project_out(j, out, (2, 3))

    out = late(W_BLOCKS - DEPTH, out)
    out = lax.fori_loop(W_BLOCKS - DEPTH, W_BLOCKS, early, out)
    out = lax.fori_loop(W_BLOCKS - DEPTH + 1, W_BLOCKS, late, out)
    o_ref[...] = out.astype(o_ref.dtype)


def _kernel(*refs):
    pl.run_scoped(functools.partial(_stream, *refs),
                  pltpu.SemaphoreType.DMA((SLOTS,)), pltpu.SemaphoreType.DMA((SLOTS + 1,)))


@jax.jit
def pallas_gated_mix__mha_block_cached__swiglu_ffn__decode_kernel(
    A_x: jax.Array,
    A_k_cache: jax.Array,
    A_v_cache: jax.Array,
    A_wq: jax.Array,
    A_wo: jax.Array,
    B_x: jax.Array,
    B_w_gate: jax.Array,
    B_w_up: jax.Array,
    B_w_down: jax.Array,
    gate_w: jax.Array,
):
    del B_x
    hbm = pl.BlockSpec(memory_space=pltpu.HBM)
    out = pl.pallas_call(
        _kernel,
        name="gated_mix_decode",
        out_shape=jax.ShapeDtypeStruct((B, D), A_x.dtype),
        in_specs=[hbm] * 9,
        out_specs=pl.BlockSpec(memory_space=pltpu.VMEM),
        scratch_shapes=[
            pltpu.VMEM((SLOTS, G, T, DH), BF16),
            pltpu.VMEM((V_SLOTS, G // 2, 2, T, DH), BF16),
            pltpu.VMEM((8, D // 8, H * DH), BF16),
            pltpu.VMEM((4, H * DH // 4, D), BF16),
            pltpu.VMEM((FFN_BANDS * DH, D), BF16),
            pltpu.VMEM((FFN_BANDS * DH, D), BF16),
            pltpu.VMEM((FFN_BANDS * DH, D), BF16),
            pltpu.VMEM((B, D), BF16),
            pltpu.VMEM((D // DH, DH), BF16),
            pltpu.VMEM((B, H, DH), F32),
            pltpu.VMEM((B, H, DH), F32),
            pltpu.VMEM((G, D), F32),
            pltpu.SMEM((1,), jnp.int32),
        ],
        compiler_params=pltpu.CompilerParams(vmem_limit_bytes=40 * 1024 * 1024),
    )(
        A_x.reshape(B, D),
        A_k_cache.reshape(B * H, SK, DH),
        A_v_cache.reshape(B * H // 2, 2, SK, DH),
        A_wq.reshape(8, D // 8, H * DH),
        A_wo.reshape(4, H * DH // 4, D),
        B_w_gate.T,
        B_w_up.T,
        B_w_down,
        gate_w.reshape(D // DH, DH),
    )
    return out.reshape(B, 1, D)
```

```python
import functools
import math

import jax
import jax.numpy as jnp
from jax import lax
from jax.experimental import pallas as pl
from jax.experimental.pallas import tpu as pltpu

B, D, H, SK, DH, F = 4, 512, 32, 4096, 128, 1376

T = 128
G = 8
KEY_BLOCKS = SK // T
GROUPS = B * H // G
KV_BLOCKS = GROUPS * KEY_BLOCKS
W_BLOCKS = 8
FFN_ROWS = 160
FFN_BANDS = -(-F // DH)

DEPTH = 5
SLOTS = 8
K_ORDER = (7, 2, 5, 4, 6, 3, 0, 1)
V_ORDER = (2, 1, 3, 0)
PAUSE = 10
IDLE_PAUSE = 13

EXP2_SCALE = DH ** -0.5 * math.log2(math.e)
F32, BF16 = jnp.float32, jnp.bfloat16


def _hint(v, m):
    return v if isinstance(v, int) else pl.multiple_of(v, m)


def _dot(a, b):
    return jnp.dot(a, b, preferred_element_type=F32)


def _dot_nt(a, b):
    return lax.dot_general(a, b, (((1,), (1,)), ((), ())), preferred_element_type=F32)


def _start(copies, priority):
    for c in copies:
        pltpu.make_async_copy(*c).start(priority=priority)


def _wait(copies):
    for c in copies:
        pltpu.make_async_copy(*c).wait()


def _stream(x_hbm, k_hbm, v_hbm, wq_hbm, wo_hbm, wg_hbm, wu_hbm, wd_hbm, gw_hbm, o_ref,
            k_buf, v_buf, wq, wo, wg, wu, wd, x_ref, gw_ref, q_all, o_all, ffn_acc, tick_ref,
            sem_small, sem_bulk):

    def wq_block(j):
        def part(which, half, sem):
            at = (which, pl.ds(_hint(j * 8, 8), 8), pl.ds(half * (H * DH // 2), H * DH // 2))
            return wq_hbm.at[at], wq.at[at], sem.at[j & (SLOTS - 1)]

        small = [part(i % 4, i // 4, sem_small) for i in range(8)]
        return small, [part(pl.ds(4, 4), half, sem_bulk) for half in range(2)]

    def ffn_block(j):
        def part(src, dst, first, count, sem):
            rows = pl.ds(_hint(j * FFN_ROWS + first, 32), count)
            return src.at[rows], dst.at[rows], sem.at[j & (SLOTS - 1)]

        small = []
        for u in range(5):
            small.append(part(wg_hbm, wg, 32 * u, 32, sem_small))
            if u < 3:
                small.append(part(wd_hbm, wd, 32 * u, 32, sem_small))
        return small, [part(wu_hbm, wu, 0, FFN_ROWS, sem_bulk), part(wd_hbm, wd, 96, FFN_ROWS - 96, sem_bulk)]

    def kv_block(n):
        slot, g = n & (SLOTS - 1), lax.div(n, KEY_BLOCKS)
        kb = (n & (KEY_BLOCKS - 4)) + ((n & 1) << 1) + ((n >> 1) & 1)
        keys = pl.ds(_hint(kb * T, T), T)
        small = [(k_hbm.at[g * G + i, keys], k_buf.at[slot, i], sem_small.at[slot]) for i in K_ORDER]
        bulk = [(v_hbm.at[pl.ds(g * G + 2 * u, 2), keys], v_buf.at[slot, pl.ds(2 * u, 2)], sem_bulk.at[slot])
                for u in V_ORDER]
        return small, bulk

    def wo_block(j):
        def part(which, u, sem):
            rows = pl.ds(_hint(j * DH + 32 * u, 32), 32)
            return wo_hbm.at[which, rows], wo.at[which, rows], sem.at[j & (SLOTS - 1)]

        small = [part(i % 2, i // 2, sem_small) for i in range(8)]
        return small, [part(pl.ds(2, 2), u, sem_bulk) for u in range(4)]

    last_rows = pl.ds(W_BLOCKS * FFN_ROWS, F - W_BLOCKS * FFN_ROWS)
    rest = [(x_hbm, x_ref), (gw_hbm, gw_ref)]
    rest += [(src.at[last_rows], dst.at[last_rows]) for src, dst in ((wg_hbm, wg), (wu_hbm, wu), (wd_hbm, wd))]
    rest = [(src, dst, sem_bulk.at[SLOTS]) for src, dst in rest]

    def start_spaced(copies, steps, tick):
        _start(copies[:1], 0)
        for c in copies[1:]:
            tick = lax.fori_loop(0, steps, lambda _, t: (t * 3 + 1) & 0xFFFF, tick)
            _start([c], 0)
        tick_ref[0] = tick

    def wait_block(block, j):
        small, bulk = block(j)
        if block is kv_block:
            slot = j & (SLOTS - 1)
            small = [(k_buf.at[slot], k_buf.at[slot], sem_small.at[slot])]
        _wait(bulk + small)

    def consume(first, stop, block, ahead, compute, carry):
        def step(j, carry):
            wait_block(block, j)
            small, bulk = ahead(j + DEPTH)
            _start(bulk, 1)
            if compute is None:
                return start_spaced(small, IDLE_PAUSE, j)
            _start(small[:1], 0)
            carry = compute(j, carry)
            start_spaced(small[1:], PAUSE, j)
            return carry

        return lax.fori_loop(first, stop, step, carry)

    def phase(count, block, following, compute, carry):
        carry = consume(0, count - DEPTH, block, block, compute, carry)
        return consume(count - DEPTH, count, block, lambda u: following(u - count), compute, carry)

    for j in range(DEPTH):
        _start(wq_block(j)[1], 1)
    _start(rest, 1)

    start_spaced(sum((wq_block(j)[0] for j in range(DEPTH)), []), IDLE_PAUSE, jnp.int32(0))

    for w in (wg, wu, wd):
        w[pl.ds(F, FFN_BANDS * DH - F), :] = jnp.zeros((FFN_BANDS * DH - F, D), BF16)
    v_buf[SLOTS - 1] = jnp.zeros(v_buf.shape[1:], BF16)
    ffn_acc[...] = jnp.zeros((G, D), F32)

    phase(W_BLOCKS, wq_block, ffn_block, None, None)
    _wait(rest)

    def load_x():
        x = x_ref[...].astype(F32)
        return jnp.concatenate([x, x], axis=0).astype(BF16)

    def project_q(j, _):
        w = wq[:, :, pl.ds(_hint(j * (4 * DH), 4 * DH), 4 * DH)].reshape(D, 4 * DH)
        q = _dot(load_x(), w)
        for i in range(4):
            q_all[:, pl.ds(4 * j + i, 1), :] = q[:B, i * DH:(i + 1) * DH].reshape(B, 1, DH)

    phase(W_BLOCKS, ffn_block, kv_block, project_q, None)

    row = lax.broadcasted_iota(jnp.int32, (G, DH), 0)

    def heads(g):
        return lax.div(g, H // G), pl.ds(_hint((g & (H // G - 1)) * G, G), G)

    def per_head(product):
        out = product(0)
        for i in range(1, G):
            out = jnp.where(row == i, product(i), out)
        return out

    def accumulate(n, m, total, acc, s):
        m_new = jnp.maximum(m, jnp.max(s, axis=1, keepdims=True))
        alpha = jnp.exp2((m - m_new) * EXP2_SCALE)
        e = jnp.exp2((s - m_new) * EXP2_SCALE)
        p = e.astype(BF16)
        pv = per_head(lambda i: _dot(p, v_buf[n & (SLOTS - 1), i]))
        return m_new, total * alpha + e, acc * alpha + pv

    def finish_group(g, total, acc):
        o_all[heads(g)] = acc / jnp.sum(total, axis=1, keepdims=True)

    def ffn_band(j):
        rows = pl.ds(_hint(j * DH, DH), DH)
        x = load_x()
        gate, up = _dot_nt(x, wg[rows, :]), _dot_nt(x, wu[rows, :])
        hidden = (gate * jax.nn.sigmoid(gate) * up).astype(BF16)
        ffn_acc[...] += _dot(hidden, wd[rows, :])

    def attend(n, carry):
        m, total, acc, s_prev = carry
        g, kb = lax.div(n, KEY_BLOCKS), n & (KEY_BLOCKS - 1)
        m, total, acc = accumulate(n + SLOTS - 1, m, total, acc, s_prev)
        q = q_all[heads(g)].astype(BF16)
        s = per_head(lambda i: _dot_nt(q, k_buf[n & (SLOTS - 1), i]))
        pl.when((kb == 0) & (n > 0))(lambda: finish_group(g - 1, total, acc))
        pl.when((kb == KEY_BLOCKS // 2) & (g < FFN_BANDS))(lambda: ffn_band(g))
        fresh = kb == 0
        return jnp.where(fresh, -jnp.inf, m), jnp.where(fresh, 0.0, total), jnp.where(fresh, 0.0, acc), s

    zero = ffn_acc[:, :DH]
    m, total, acc, s = phase(KV_BLOCKS, kv_block, wo_block, attend, (zero,) * 4)
    _, total, acc = accumulate(KV_BLOCKS - 1, m, total, acc, s)
    finish_group(jnp.int32(GROUPS - 1), total, acc)

    x, gw = x_ref[...].astype(F32), gw_ref[...].astype(F32)
    logit = sum(x[:, r * DH:(r + 1) * DH] * gw[r:r + 1, :] for r in range(D // DH))
    mix = jax.nn.sigmoid(jnp.sum(logit, axis=1, keepdims=True))

    def project_out(j, out, which=(0, 1, 2, 3)):
        rows = pl.ds(_hint(j * DH, DH), DH)
        attn = sum(_dot(o_all[:, pl.ds(8 * i + j, 1), :].reshape(B, DH).astype(BF16), wo[i, rows, :]) for i in which)
        return out + mix * attn

    out = (1.0 - mix) * ffn_acc[:B, :]
    out = consume(0, W_BLOCKS - DEPTH, wo_block, wo_block, project_out, out)

    def early(j, out):
        _wait(wo_block(j)[0])
        return project_out(j, out, (0, 1))

    def late(j, out):
        _wait(wo_block(j)[1])
        return project_out(j, out, (2, 3))

    out = late(W_BLOCKS - DEPTH, out)
    out = lax.fori_loop(W_BLOCKS - DEPTH, W_BLOCKS, early, out)
    out = lax.fori_loop(W_BLOCKS - DEPTH + 1, W_BLOCKS, late, out)
    o_ref[...] = out.astype(o_ref.dtype)


def _kernel(*refs):
    pl.run_scoped(functools.partial(_stream, *refs),
                  pltpu.SemaphoreType.DMA((SLOTS,)), pltpu.SemaphoreType.DMA((SLOTS + 1,)))


@jax.jit
def pallas_gated_mix__mha_block_cached__swiglu_ffn__decode_kernel(
    A_x: jax.Array,
    A_k_cache: jax.Array,
    A_v_cache: jax.Array,
    A_wq: jax.Array,
    A_wo: jax.Array,
    B_x: jax.Array,
    B_w_gate: jax.Array,
    B_w_up: jax.Array,
    B_w_down: jax.Array,
    gate_w: jax.Array,
):
    del B_x
    hbm = pl.BlockSpec(memory_space=pltpu.HBM)
    out = pl.pallas_call(
        _kernel,
        name="gated_mix_decode",
        out_shape=jax.ShapeDtypeStruct((B, D), A_x.dtype),
        in_specs=[hbm] * 9,
        out_specs=pl.BlockSpec(memory_space=pltpu.VMEM),
        scratch_shapes=[
            pltpu.VMEM((SLOTS, G, T, DH), BF16),
            pltpu.VMEM((SLOTS, G, T, DH), BF16),
            pltpu.VMEM((8, D // 8, H * DH), BF16),
            pltpu.VMEM((4, H * DH // 4, D), BF16),
            pltpu.VMEM((FFN_BANDS * DH, D), BF16),
            pltpu.VMEM((FFN_BANDS * DH, D), BF16),
            pltpu.VMEM((FFN_BANDS * DH, D), BF16),
            pltpu.VMEM((B, D), BF16),
            pltpu.VMEM((D // DH, DH), BF16),
            pltpu.VMEM((B, H, DH), F32),
            pltpu.VMEM((B, H, DH), F32),
            pltpu.VMEM((G, D), F32),
            pltpu.SMEM((1,), jnp.int32),
        ],
        compiler_params=pltpu.CompilerParams(vmem_limit_bytes=40 * 1024 * 1024),
    )(
        A_x.reshape(B, D),
        A_k_cache.reshape(B * H, SK, DH),
        A_v_cache.reshape(B * H, SK, DH),
        A_wq.reshape(8, D // 8, H * DH),
        A_wo.reshape(4, H * DH // 4, D),
        B_w_gate.T,
        B_w_up.T,
        B_w_down,
        gate_w.reshape(D // DH, DH),
    )
    return out.reshape(B, 1, D)
```
